```python
import jax
import jax.numpy as jnp

def _softmax(x, axis=-1):
    return jax.nn.softmax(x, axis=axis)

def _gelu(x):
    return jax.nn.gelu(x, approximate=True)

def _silu(x):
    return jax.nn.silu(x)

def _sigmoid(x):
    return jax.nn.sigmoid(x)

def _layernorm(x, axis=-1, eps=1e-05):
    m = jnp.mean(x, axis=axis, keepdims=True)
    v = jnp.var(x, axis=axis, keepdims=True)
    return (x - m) / jnp.sqrt(v + eps)

def _scatter_add(tgt, idx, src, axis=0):
    return tgt.at[idx].add(src)

def _segment_sum(src, seg, n):
    return jax.ops.segment_sum(src, seg, n)

class _Rng:

    def __init__(self, key):
        self._k = key

    def _next(self):
        self._k, sub = jax.random.split(self._k)
        return sub

    def normal(self, shape):
        return jax.random.normal(self._next(), shape, dtype=jnp.bfloat16)

    def randint(self, lo, hi, shape):
        return jax.random.randint(self._next(), shape, lo, hi, dtype=jnp.int32)

    def uniform(self, shape, lo=0.0, hi=1.0):
        return jax.random.uniform(self._next(), shape, jnp.bfloat16, lo, hi)

    def permutation(self, n):
        return jax.random.permutation(self._next(), n)
kernel_name = 'adaLN_cond__sliding_block_cached__glu_gated_bilinear__decode'

def setup_inputs():
    _rng = _Rng(jax.random.key(int.from_bytes(__import__("os").urandom(4), "little")))
    _w = lambda a: (lambda t: t.astype(jnp.bfloat16) if jnp.issubdtype(t.dtype, jnp.floating) else t)(jnp.asarray(a))

    def _A_setup():
        B, Sq, D = (1, 1, 640)
        Hq, Hkv, Sk, Dh = (32, 32, 32768, 192)
        assert Hq % Hkv == 0, (Hq, Hkv)
        return {'x': _w((lambda *s: _rng.normal(s) * 0.05)(B, Sq, D)), 'k_cache': _w((lambda *s: _rng.normal(s) * 0.05)(B, Hkv, Sk, Dh)), 'v_cache': _w((lambda *s: _rng.normal(s) * 0.05)(B, Hkv, Sk, Dh)), 'wq': _w((lambda *s: _rng.normal(s) * 0.05)(D, Hq * Dh) * D ** (-0.5)), 'wo': _w((lambda *s: _rng.normal(s) * 0.05)(Hq * Dh, D) * (Hq * Dh) ** (-0.5))}
    _A_in = _A_setup()

    def _B_setup():
        B, S, D, F = (1, 1, 640, 1536)
        return {'x': _w((lambda *s: _rng.normal(s) * 0.05)(B, S, D)), 'w_gate': _w((lambda *s: _rng.normal(s) * 0.05)(D, F) * D ** (-0.5)), 'w_up': _w((lambda *s: _rng.normal(s) * 0.05)(D, F) * D ** (-0.5)), 'w_down': _w((lambda *s: _rng.normal(s) * 0.05)(F, D) * F ** (-0.5))}
    _B_in = _B_setup()
    return {'A_x': _A_in['x'], 'A_k_cache': _A_in['k_cache'], 'A_v_cache': _A_in['v_cache'], 'A_wq': _A_in['wq'], 'A_wo': _A_in['wo'], 'B_x': _B_in['x'], 'B_w_gate': _B_in['w_gate'], 'B_w_up': _B_in['w_up'], 'B_w_down': _B_in['w_down'], 'c': _w((lambda *s: _rng.normal(s) * 0.05)(1, 640)), 'w_mod': _w((lambda *s: _rng.normal(s) * 0.05)(640, 6 * 640) * 640 ** (-0.5))}

def reference(A_x, A_k_cache, A_v_cache, A_wq, A_wo, B_x, B_w_gate, B_w_up, B_w_down, c, w_mod):

    def _A_ref(x, k_cache, v_cache, wq, wo):
        B, Sq, D = x.shape
        Hq, Dh = (32, 192)
        Hkv, Sk = (k_cache.shape[1], k_cache.shape[2])
        W = min(4096, max(256, Sk // 4))
        rep = Hq // Hkv
        q = (lambda x, *d: x.transpose(*d))((x @ wq).reshape(B, Sq, Hq, Dh), 0, 2, 1, 3)
        k = jnp.repeat(k_cache[:, :, Sk - W:, :], rep, axis=1)
        v = jnp.repeat(v_cache[:, :, Sk - W:, :], rep, axis=1)
        scores = jnp.einsum('bhqd,bhkd->bhqk', q, k) * Dh ** (-0.5)
        p = _softmax(scores, axis=-1)
        o = jnp.einsum('bhqk,bhkd->bhqd', p, v)
        return (lambda x, *d: x.transpose(*d))(o, 0, 2, 1, 3).reshape(B, Sq, Hq * Dh) @ wo

    def _B_ref(x, w_gate, w_up, w_down):
        g = jnp.einsum('bsd,df->bsf', x, w_gate)
        u = jnp.einsum('bsd,df->bsf', x, w_up)
        h = g * u
        return jnp.einsum('bsf,fd->bsd', h, w_down)
    x = A_x
    mod = (_silu(c) @ w_mod).reshape(c.shape[0], 6, 1, -1)
    sa, ca, ga, sb, cb, gb = (mod[:, 0].copy(), mod[:, 1].copy(), mod[:, 2].copy(), mod[:, 3].copy(), mod[:, 4].copy(), mod[:, 5].copy())
    h = _layernorm(x, axis=-1) * (1 + ca) + sa
    x = x + ga * _A_ref(h, A_k_cache, A_v_cache, A_wq, A_wo)
    h = _layernorm(x, axis=-1) * (1 + cb) + sb
    x = x + gb * _B_ref(h, B_w_gate, B_w_up, B_w_down)
    return x
```

```python
import functools
import jax
import jax.numpy as jnp
from jax import lax
import jax.experimental.pallas as pl
import jax.experimental.pallas.tpu as pltpu

D = 640
H = 32
DH = 192
SK = 32768
W = 4096
F = 1536
G = 2
NG = H // G
GD = G * DH
NB = 4
EPS = 1e-5


def _ln(x):
    m = jnp.mean(x, axis=-1, keepdims=True)
    xc = x - m
    v = jnp.mean(xc * xc, axis=-1, keepdims=True)
    return xc * lax.rsqrt(v + EPS)


def _mm(a, b):
    return jnp.dot(a, b, preferred_element_type=jnp.float32)


def kernel(x_hbm, c_hbm, kT_hbm, vT_hbm, wq_hbm, wo_hbm, wg_hbm, wu_hbm, wd_hbm, wmod_hbm,
           out_ref,
           x_buf, c_buf, wmod_buf, wq_buf, wo_buf, wg_buf, wu_buf, wd_buf, k_buf, v_buf, q_buf,
           wsem, ksem, vsem):
    def kv_copies(g, slot):
        r = pl.ds(pl.multiple_of(g * GD, GD), GD)
        ck = pltpu.make_async_copy(kT_hbm.at[r, pl.ds(SK - W, W)], k_buf.at[slot], ksem.at[slot])
        cv = pltpu.make_async_copy(vT_hbm.at[r, pl.ds(SK - W, W)], v_buf.at[slot], vsem.at[slot])
        return ck, cv

    cp_x = pltpu.make_async_copy(x_hbm, x_buf, wsem.at[0])
    cp_c = pltpu.make_async_copy(c_hbm, c_buf, wsem.at[1])
    cp_mod = pltpu.make_async_copy(wmod_hbm, wmod_buf, wsem.at[2])
    cp_wq = pltpu.make_async_copy(wq_hbm, wq_buf, wsem.at[3])
    cp_wo = pltpu.make_async_copy(wo_hbm, wo_buf, wsem.at[4])
    cp_wg = pltpu.make_async_copy(wg_hbm, wg_buf, wsem.at[5])
    cp_wu = pltpu.make_async_copy(wu_hbm, wu_buf, wsem.at[6])
    cp_wd = pltpu.make_async_copy(wd_hbm, wd_buf, wsem.at[7])
    cp_x.start(); cp_c.start(); cp_mod.start(); cp_wq.start()
    for s in range(NB):
        ck, cv = kv_copies(s, s)
        ck.start(); cv.start()
    cp_wo.start()

    cp_x.wait(); cp_c.wait(); cp_mod.wait()
    x = x_buf[...].astype(jnp.float32)
    c = c_buf[...].astype(jnp.float32)
    sc = (c * jax.nn.sigmoid(c)).astype(jnp.bfloat16)
    mod = _mm(sc, wmod_buf[...])
    sa, ca, ga, sb, cb, gb = [mod[:, i * D:(i + 1) * D] for i in range(6)]
    h = (_ln(x) * (1.0 + ca) + sa).astype(jnp.bfloat16)
    cp_wq.wait()
    q = _mm(h, wq_buf[...]) * (DH ** -0.5)
    q_buf[...] = jnp.broadcast_to(q, (8, H * DH))
    cp_wo.wait()

    row = lax.broadcasted_iota(jnp.int32, (8, GD), 0)
    lane = lax.broadcasted_iota(jnp.int32, (8, GD), 1)
    diag = (lane // DH) == row

    def body(g, acc):
        slot = g % NB
        ck, cv = kv_copies(g, slot)
        off = pl.multiple_of(g * GD, GD)
        qg = jnp.where(diag, q_buf[:, pl.ds(off, GD)], 0.0).astype(jnp.bfloat16)
        ck.wait()
        s = _mm(qg, k_buf[slot])
        m = jnp.max(s, axis=-1, keepdims=True)
        p = jnp.exp(s - m)
        l = jnp.sum(p, axis=-1, keepdims=True)
        cv.wait()
        o = lax.dot_general(p.astype(jnp.bfloat16), v_buf[slot], (((1,), (1,)), ((), ())),
                            preferred_element_type=jnp.float32)

        @pl.when(g + NB < NG)
        def _():
            nk, nv = kv_copies(g + NB, slot)
            nk.start(); nv.start()

        @pl.when(g + NB == NG)
        def _():
            cp_wg.start(); cp_wu.start(); cp_wd.start()

        o = jnp.where(diag, o / l, 0.0).astype(jnp.bfloat16)
        return acc + _mm(o, wo_buf[pl.ds(off, GD), :])

    acc = lax.fori_loop(0, NG, body, jnp.zeros((8, D), jnp.float32))
    attn = jnp.sum(acc, axis=0, keepdims=True)
    x1 = x + ga * attn
    h2 = (_ln(x1) * (1.0 + cb) + sb).astype(jnp.bfloat16)
    cp_wg.wait()
    gt = _mm(h2, wg_buf[...])
    cp_wu.wait()
    up = _mm(h2, wu_buf[...])
    hd = (gt * up).astype(jnp.bfloat16)
    cp_wd.wait()
    ff = _mm(hd, wd_buf[...])
    out_ref[...] = (x1 + gb * ff).astype(out_ref.dtype)


@jax.jit
def pallas_adaLN_cond__sliding_block_cached__glu_gated_bilinear__decode_kernel(A_x, A_k_cache, A_v_cache, A_wq, A_wo, B_x, B_w_gate, B_w_up, B_w_down, c, w_mod):
    kT = jnp.swapaxes(A_k_cache, 2, 3).reshape(H * DH, SK)
    vT = jnp.swapaxes(A_v_cache, 2, 3).reshape(H * DH, SK)
    x2 = A_x.reshape(1, D)
    any_spec = pl.BlockSpec(memory_space=pl.ANY)
    out = pl.pallas_call(
        kernel,
        in_specs=[any_spec] * 10,
        out_specs=pl.BlockSpec(memory_space=pltpu.VMEM),
        out_shape=jax.ShapeDtypeStruct((1, D), A_x.dtype),
        scratch_shapes=[
            pltpu.VMEM((1, D), jnp.bfloat16), pltpu.VMEM((1, D), jnp.bfloat16),
            pltpu.VMEM((D, 6 * D), jnp.bfloat16), pltpu.VMEM((D, H * DH), jnp.bfloat16),
            pltpu.VMEM((H * DH, D), jnp.bfloat16), pltpu.VMEM((D, F), jnp.bfloat16),
            pltpu.VMEM((D, F), jnp.bfloat16), pltpu.VMEM((F, D), jnp.bfloat16),
            pltpu.VMEM((NB, GD, W), jnp.bfloat16), pltpu.VMEM((NB, GD, W), jnp.bfloat16),
            pltpu.VMEM((8, H * DH), jnp.float32),
            pltpu.SemaphoreType.DMA((8,)), pltpu.SemaphoreType.DMA((NB,)), pltpu.SemaphoreType.DMA((NB,)),
        ],
        compiler_params=pltpu.CompilerParams(vmem_limit_bytes=100 * 1024 * 1024),
    )(x2, c, kT, vT, A_wq, A_wo, B_w_gate, B_w_up, B_w_down, w_mod)
    return out.reshape(1, 1, D)
```

```python
import jax
import jax.numpy as jnp
from jax import lax
import jax.experimental.pallas as pl
import jax.experimental.pallas.tpu as pltpu

D = 640
H = 32
DH = 192
SK = 32768
W = 4096
F = 1536
G = 2
NG = H // G
GD = G * DH
NB = 4
EPS = 1e-5
FC = 128
NF = F // FC


def _ln(x):
    m = jnp.mean(x, axis=-1, keepdims=True)
    xc = x - m
    v = jnp.mean(xc * xc, axis=-1, keepdims=True)
    return xc * lax.rsqrt(v + EPS)


def _mm(a, b):
    return jnp.dot(a, b, preferred_element_type=jnp.float32)


def kernel(x_hbm, c_hbm, kT_hbm, vT_hbm, wq_hbm, wo_hbm, wg_hbm, wu_hbm, wd_hbm, wmod_hbm,
           out_ref,
           x_buf, c_buf, wmod_buf, wq_buf, wo_buf, wg_buf, wu_buf, wd_buf, k_buf, v_buf, mod_buf, hd_buf,
           wsem, ksem, vsem, osem, dsem):
    def kv_copies(g, slot):
        r = pl.ds(pl.multiple_of(g * GD, GD), GD)
        ck = pltpu.make_async_copy(kT_hbm.at[r, pl.ds(SK - W, W)], k_buf.at[slot], ksem.at[slot])
        cv = pltpu.make_async_copy(vT_hbm.at[r, pl.ds(SK - W, W)], v_buf.at[slot], vsem.at[slot])
        co = pltpu.make_async_copy(wo_hbm.at[r, :], wo_buf.at[slot], osem.at[slot])
        return ck, cv, co

    def wd_copy(j):
        r = pl.ds(pl.multiple_of(j * FC, FC), FC)
        return pltpu.make_async_copy(wd_hbm.at[r, :], wd_buf.at[r, :], dsem.at[j])

    cp_x = pltpu.make_async_copy(x_hbm, x_buf, wsem.at[0])
    cp_c = pltpu.make_async_copy(c_hbm, c_buf, wsem.at[1])
    cp_mod = pltpu.make_async_copy(wmod_hbm, wmod_buf, wsem.at[2])
    cp_wq = pltpu.make_async_copy(wq_hbm, wq_buf, wsem.at[3])
    cp_wg = pltpu.make_async_copy(wg_hbm, wg_buf, wsem.at[4])
    cp_wu = pltpu.make_async_copy(wu_hbm, wu_buf, wsem.at[5])
    cp_x.start(); cp_c.start(); cp_mod.start(); cp_wq.start()

    @pl.loop(0, NB)
    def _(s):
        ck, cv, co = kv_copies(s, s)
        ck.start(); cv.start(); co.start()

    cp_x.wait(); cp_c.wait()
    x = x_buf[...].astype(jnp.float32)
    c = c_buf[...].astype(jnp.float32)
    sc = jnp.broadcast_to((c * jax.nn.sigmoid(c)).astype(jnp.bfloat16), (8, D))
    cp_mod.wait()

    def mod_body(j, _):
        off = pl.multiple_of(j * D, D)
        mod_buf[j] = _mm(sc, wmod_buf[:, pl.ds(off, D)])
        return 0
    lax.fori_loop(0, 6, mod_body, 0)

    sa = mod_buf[0][0:1]; ca = mod_buf[1][0:1]
    h = jnp.broadcast_to((_ln(x) * (1.0 + ca) + sa).astype(jnp.bfloat16), (8, D))
    cp_wq.wait()

    row = lax.broadcasted_iota(jnp.int32, (8, GD), 0)
    lane = lax.broadcasted_iota(jnp.int32, (8, GD), 1)
    diag = (lane // DH) == row

    def body(g, acc):
        slot = g % NB
        ck, cv, co = kv_copies(g, slot)
        off = pl.multiple_of(g * GD, GD)
        q = _mm(h, wq_buf[:, pl.ds(off, GD)]) * (DH ** -0.5)
        qg = jnp.where(diag, q, 0.0).astype(jnp.bfloat16)
        ck.wait()
        s = _mm(qg, k_buf[slot])
        m = jnp.max(s, axis=-1, keepdims=True)
        p = jnp.exp(s - m)
        l = jnp.sum(p, axis=-1, keepdims=True)
        cv.wait()
        o = lax.dot_general(p.astype(jnp.bfloat16), v_buf[slot], (((1,), (1,)), ((), ())),
                            preferred_element_type=jnp.float32)
        o = jnp.where(diag, o / l, 0.0).astype(jnp.bfloat16)
        co.wait()
        acc = acc + _mm(o, wo_buf[slot])

        @pl.when(g + NB < NG)
        def _():
            nk, nv, no = kv_copies(g + NB, slot)
            nk.start(); nv.start(); no.start()

        @pl.when(g + NB == NG)
        def _():
            cp_wg.start(); cp_wu.start()

            @pl.loop(0, NF)
            def _(j):
                wd_copy(j).start()
        return acc

    acc = lax.fori_loop(0, NG, body, jnp.zeros((8, D), jnp.float32))
    attn = jnp.sum(acc, axis=0, keepdims=True)
    ga = mod_buf[2][0:1]; sb = mod_buf[3][0:1]; cb = mod_buf[4][0:1]; gb = mod_buf[5][0:1]
    x1 = x + ga * attn
    h2 = jnp.broadcast_to((_ln(x1) * (1.0 + cb) + sb).astype(jnp.bfloat16), (8, D))
    cp_wg.wait()
    gt = _mm(h2, wg_buf[...])
    cp_wu.wait()
    up = _mm(h2, wu_buf[...])
    hd_buf[...] = (gt * up).astype(jnp.bfloat16)

    def fbody(j, ff):
        off = pl.multiple_of(j * FC, FC)
        wd_copy(j).wait()
        return ff + _mm(hd_buf[:, pl.ds(off, FC)], wd_buf[pl.ds(off, FC), :])
    ff = lax.fori_loop(0, NF, fbody, jnp.zeros((8, D), jnp.float32))
    out_ref[...] = (x1 + gb * ff[0:1]).astype(out_ref.dtype)


@jax.jit
def pallas_adaLN_cond__sliding_block_cached__glu_gated_bilinear__decode_kernel(A_x, A_k_cache, A_v_cache, A_wq, A_wo, B_x, B_w_gate, B_w_up, B_w_down, c, w_mod):
    kT = jnp.swapaxes(A_k_cache, 2, 3).reshape(H * DH, SK)
    vT = jnp.swapaxes(A_v_cache, 2, 3).reshape(H * DH, SK)
    x2 = A_x.reshape(1, D)
    any_spec = pl.BlockSpec(memory_space=pl.ANY)
    out = pl.pallas_call(
        kernel,
        in_specs=[any_spec] * 10,
        out_specs=pl.BlockSpec(memory_space=pltpu.VMEM),
        out_shape=jax.ShapeDtypeStruct((1, D), A_x.dtype),
        scratch_shapes=[
            pltpu.VMEM((1, D), jnp.bfloat16), pltpu.VMEM((1, D), jnp.bfloat16),
            pltpu.VMEM((D, 6 * D), jnp.bfloat16), pltpu.VMEM((D, H * DH), jnp.bfloat16),
            pltpu.VMEM((NB, GD, D), jnp.bfloat16), pltpu.VMEM((D, F), jnp.bfloat16),
            pltpu.VMEM((D, F), jnp.bfloat16), pltpu.VMEM((F, D), jnp.bfloat16),
            pltpu.VMEM((NB, GD, W), jnp.bfloat16), pltpu.VMEM((NB, GD, W), jnp.bfloat16),
            pltpu.VMEM((6, 8, D), jnp.float32), pltpu.VMEM((8, F), jnp.bfloat16),
            pltpu.SemaphoreType.DMA((6,)), pltpu.SemaphoreType.DMA((NB,)), pltpu.SemaphoreType.DMA((NB,)),
            pltpu.SemaphoreType.DMA((NB,)), pltpu.SemaphoreType.DMA((NF,)),
        ],
        compiler_params=pltpu.CompilerParams(vmem_limit_bytes=100 * 1024 * 1024),
    )(x2, c, kT, vT, A_wq, A_wo, B_w_gate, B_w_up, B_w_down, w_mod)
    return out.reshape(1, 1, D)
```

```python
import functools
import jax
import jax.numpy as jnp
from jax import lax
import jax.experimental.pallas as pl
import jax.experimental.pallas.tpu as pltpu

D = 640
H = 32
DH = 192
SK = 32768
W = 4096
F = 1536
G = 2
NG = H // G
GD = G * DH
EPS = 1e-5


def _ln(x):
    m = jnp.mean(x, axis=-1, keepdims=True)
    xc = x - m
    v = jnp.mean(xc * xc, axis=-1, keepdims=True)
    return xc * lax.rsqrt(v + EPS)


def _mm(a, b):
    return jnp.dot(a, b, preferred_element_type=jnp.float32)


def _ds(i, n):
    return pl.ds(pl.multiple_of(i * n, n), n)


def kernel(x_hbm, c_hbm, kT_hbm, vT_hbm, wq_hbm, wo_hbm, wg_hbm, wu_hbm, wd_hbm, wmod_hbm,
           out_ref,
           x_buf, c_buf, wmod_buf, wq_buf, wo_buf, wg_buf, wu_buf, wd_buf, k_buf, v_buf, mod_buf,
           q_buf, s_buf, hd_buf, ff_buf, t_buf, sem, *, LR, KW, splits, KB, UPI):
    NKB = W // KB

    def cols2(src, dst, r, nr, w0, s):
        n = src.shape[1]
        rows = _ds(r, nr)
        return [(pltpu.make_async_copy(src.at[rows, pl.ds(0, w0)], dst.at[rows, pl.ds(0, w0)], s), 0),
                (pltpu.make_async_copy(src.at[rows, pl.ds(w0, n - w0)], dst.at[rows, pl.ds(w0, n - w0)], s), 1)]

    def rows2(src, dst, r, nr, s):
        a, b = _ds(2 * r, nr), _ds(2 * r + 1, nr)
        return [(pltpu.make_async_copy(src.at[a, :], dst.at[a, :], s), 0),
                (pltpu.make_async_copy(src.at[b, :], dst.at[b, :], s), 1)]

    def u_mod(u):
        return [cols2(wmod_hbm, wmod_buf, 2 * u + j, 8, 3 * D, sem.at[0]) for j in range(2)]

    def u_wq(u):
        return [cols2(wq_hbm, wq_buf, u, 8, H * DH // 2, sem.at[1])]

    def u_wo(u):
        return [rows2(wo_hbm, wo_buf, 2 * u + j, 24, sem.at[0]) for j in range(2)]

    def u_kv(g, u):
        slot = g & 1
        s = sem.at[(g + 1) & 1]
        rows = _ds(g * (GD // 8) + u, 8)
        steps = []
        for src, dst in ((kT_hbm, k_buf), (vT_hbm, v_buf)):
            steps.append([
                (pltpu.make_async_copy(src.at[rows, pl.ds(SK - W, KW)], dst.at[slot, _ds(u, 8), pl.ds(0, KW)], s), 0),
                (pltpu.make_async_copy(src.at[rows, pl.ds(SK - W + KW, W - KW)], dst.at[slot, _ds(u, 8), pl.ds(KW, W - KW)], s), 1)])
        return steps

    def u_ffn(u):
        return [rows2(wg_hbm, wg_buf, u, 8, sem.at[1]), rows2(wu_hbm, wu_buf, u, 8, sem.at[1])]

    def start(unit):
        for step in unit:
            for cp, p in step:
                cp.start(priority=p)

    def pump(old, new):
        n = max(len(old), len(new))
        for i in range(n):
            for step in old[i * len(old) // n:(i + 1) * len(old) // n]:
                for cp, _ in step:
                    cp.wait()
            for step in new[i * len(new) // n:(i + 1) * len(new) // n]:
                for cp, p in step:
                    cp.start(priority=p)

    def pump_loop(lo, hi, old_fn, new_fn):
        if hi > lo:
            @pl.loop(lo, hi)
            def _(u):
                pump(old_fn(0), new_fn(u))

    small = [pltpu.make_async_copy(x_hbm, x_buf, sem.at[0]), pltpu.make_async_copy(c_hbm, c_buf, sem.at[0])]
    for cp in small:
        cp.start()

    @pl.loop(0, LR)
    def _(u):
        start(u_mod(u))
    pump_loop(LR, 40, u_mod, u_mod)

    pump_loop(0, LR, u_mod, u_wq)
    for cp in small:
        cp.wait()
    x = x_buf[...].astype(jnp.float32)
    c = c_buf[...].astype(jnp.float32)
    sc = jnp.broadcast_to((c * jax.nn.sigmoid(c)).astype(jnp.bfloat16), (8, D))

    @pl.loop(0, 6)
    def _(j):
        pump(u_wq(0), u_wq(LR + 2 * j))
        pump(u_wq(0), u_wq(LR + 2 * j + 1))
        mod_buf[j] = _mm(sc, wmod_buf[:, _ds(j, D)])
    pump_loop(LR + 12, 80, u_wq, u_wq)

    pump_loop(0, LR, u_wq, u_wo)
    h = jnp.broadcast_to((_ln(x) * (1.0 + mod_buf[1][0:1]) + mod_buf[0][0:1]).astype(jnp.bfloat16), (8, D))
    row = lax.broadcasted_iota(jnp.int32, (8, GD), 0)
    lane = lax.broadcasted_iota(jnp.int32, (8, GD), 1)
    diag = (lane // DH) == row

    @pl.loop(0, NG)
    def _(g):
        pump(u_wo(0), u_wo(LR + g))
        q = _mm(h, wq_buf[:, _ds(g, GD)]) * (DH ** -0.5)
        q_buf[g] = jnp.where(diag, q, 0.0)
    pump_loop(LR + NG, 64, u_wo, u_wo)

    pump_loop(0, LR, u_wo, functools.partial(u_kv, 0))
    pump_loop(LR, 48, functools.partial(u_kv, 0), functools.partial(u_kv, 0))

    def group_compute(g, acc, pump_i):
        slot = g & 1
        qg = q_buf[g].astype(jnp.bfloat16)

        def qk(i, m):
            for t in range(UPI):
                pump_i(UPI * i + t)
            s = _mm(qg, k_buf[slot, :, _ds(i, KB)])
            s_buf[:, _ds(i, KB)] = s
            for j in range(KB // 128):
                m = jnp.maximum(m, s[:, j * 128:(j + 1) * 128])
            return m
        m = lax.fori_loop(0, NKB, qk, jnp.full((8, 128), -jnp.inf, jnp.float32))
        pump_i(UPI * NKB)
        m = jnp.max(m, axis=-1, keepdims=True)

        def pv(i, carry):
            o, l = carry
            for t in range(UPI):
                pump_i(UPI * NKB + 1 + UPI * i + t)
            p = jnp.exp(s_buf[:, _ds(i, KB)] - m)
            for j in range(KB // 128):
                l = l + p[:, j * 128:(j + 1) * 128]
            o = o + lax.dot_general(p.astype(jnp.bfloat16), v_buf[slot, :, _ds(i, KB)], (((1,), (1,)), ((), ())),
                                    preferred_element_type=jnp.float32)
            return o, l
        o, l = lax.fori_loop(0, NKB, pv, (jnp.zeros((8, GD), jnp.float32), jnp.zeros((8, 128), jnp.float32)))
        pump_i(2 * UPI * NKB + 1)
        l = jnp.sum(l, axis=-1, keepdims=True)
        o = jnp.where(diag, o / l, 0.0).astype(jnp.bfloat16)
        return acc + _mm(o, wo_buf[_ds(g, GD), :])

    NC = 2 * UPI * NKB + 2

    def body(g, carry):
        acc, cnt = carry
        new = functools.partial(u_kv, g)
        old = functools.partial(u_kv, g - 1)
        pump_loop(0, LR, old, new)
        acc = group_compute(g - 1, acc, lambda i: pump(new(0), new(LR + i)))
        pump_loop(LR + NC, 48, new, new)
        return acc, cnt + 1

    acc, cnt = lax.fori_loop(1, NG, body, (jnp.zeros((8, D), jnp.float32), jnp.int32(0)))
    go = cnt == NG - 1

    pump_loop(0, LR, functools.partial(u_kv, NG - 1), u_ffn)
    acc = group_compute(NG - 1, acc, lambda i: pump(u_ffn(0), u_ffn(LR + i)))
    attn = jnp.sum(acc, axis=0, keepdims=True)
    x1 = x + mod_buf[2][0:1] * attn
    h2 = jnp.broadcast_to((_ln(x1) * (1.0 + mod_buf[4][0:1]) + mod_buf[3][0:1]).astype(jnp.bfloat16), (8, D))
    gb = mod_buf[5][0:1]
    pump_loop(LR + NC, 40, u_ffn, u_ffn)

    def wd_copy(stage):
        lo = splits[stage - 1] if stage > 0 else 0
        hi = splits[stage]
        return pltpu.make_async_copy(wd_hbm.at[lo:hi, :], wd_buf.at[lo:hi, :], sem.at[stage % 2])

    NS = len(splits)
    wd_copy(0).start(priority=1)

    @pl.loop(0, LR)
    def _(u):
        for step in u_ffn(0):
            for cp, _ in step:
                cp.wait()
    wd_copy(1).start(priority=1)

    @pl.when(go)
    def _():
        hd_buf[...] = (_mm(h2, wg_buf[...]) * _mm(h2, wu_buf[...])).astype(jnp.bfloat16)

    @pl.when(go)
    def _():
        lo, hi = splits[NS - 2], splits[NS - 1]
        R = hi - lo
        hl = hd_buf[0:1, lo:hi].astype(jnp.float32)
        eye = (lax.broadcasted_iota(jnp.int32, (R, R), 0) == lax.broadcasted_iota(jnp.int32, (R, R), 1))
        col = jnp.sum(jnp.where(eye, jnp.broadcast_to(hl, (R, R)), 0.0), axis=1, keepdims=True)
        t_buf[...] = jnp.broadcast_to(col, (R, 128))

    for stage in range(NS - 1):
        wd_copy(stage).wait()
        if stage + 2 < NS:
            wd_copy(stage + 2).start(priority=1)
        lo = splits[stage - 1] if stage > 0 else 0
        hi = splits[stage]

        @pl.when(go)
        def _():
            ff = _mm(hd_buf[:, lo:hi], wd_buf[lo:hi, :])
            if stage == 0:
                ff_buf[...] = ff
            else:
                ff_buf[...] += ff
    lo, hi = splits[NS - 2], splits[NS - 1]
    base = x1 + gb * ff_buf[0:1, :]
    wd_copy(NS - 1).wait()
    hc = t_buf[...]
    outs = []
    for j in range(D // 128):
        wv = wd_buf[lo:hi, j * 128:(j + 1) * 128].astype(jnp.float32)
        outs.append(jnp.sum(wv * hc, axis=0, keepdims=True))
    ff = jnp.concatenate(outs, axis=1)
    out_ref[...] = (base + gb * ff).astype(out_ref.dtype)


def build(LR=22, KW=2048, splits=(1024, 1408, 1536), KB=1024, UPI=2, **cp):
    R = splits[-1] - splits[-2]
    @jax.jit
    def pallas_kernel(A_x, A_k_cache, A_v_cache, A_wq, A_wo, B_x, B_w_gate, B_w_up, B_w_down, c, w_mod):
        kT = jnp.swapaxes(A_k_cache, 2, 3).reshape(H * DH, SK)
        vT = jnp.swapaxes(A_v_cache, 2, 3).reshape(H * DH, SK)
        x2 = A_x.reshape(1, D)
        any_spec = pl.BlockSpec(memory_space=pl.ANY)
        out = pl.pallas_call(
            functools.partial(kernel, LR=LR, KW=KW, splits=splits, KB=KB, UPI=UPI),
            in_specs=[any_spec] * 10,
            out_specs=pl.BlockSpec(memory_space=pltpu.VMEM),
            out_shape=jax.ShapeDtypeStruct((1, D), A_x.dtype),
            scratch_shapes=[
                pltpu.VMEM((1, D), jnp.bfloat16), pltpu.VMEM((1, D), jnp.bfloat16),
                pltpu.VMEM((D, 6 * D), jnp.bfloat16), pltpu.VMEM((D, H * DH), jnp.bfloat16),
                pltpu.VMEM((H * DH, D), jnp.bfloat16), pltpu.VMEM((D, F), jnp.bfloat16),
                pltpu.VMEM((D, F), jnp.bfloat16), pltpu.VMEM((F, D), jnp.bfloat16),
                pltpu.VMEM((2, GD, W), jnp.bfloat16), pltpu.VMEM((2, GD, W), jnp.bfloat16),
                pltpu.VMEM((6, 8, D), jnp.float32), pltpu.VMEM((NG, 8, GD), jnp.float32),
                pltpu.VMEM((8, W), jnp.float32), pltpu.VMEM((8, F), jnp.bfloat16),
                pltpu.VMEM((8, D), jnp.float32), pltpu.VMEM((R, 128), jnp.float32),
                pltpu.SemaphoreType.DMA((2,)),
            ],
            compiler_params=pltpu.CompilerParams(vmem_limit_bytes=100 * 1024 * 1024, **cp),
        )(x2, c, kT, vT, A_wq, A_wo, B_w_gate, B_w_up, B_w_down, w_mod)
        return out.reshape(1, 1, D)
    return pallas_kernel

pallas_adaLN_cond__sliding_block_cached__glu_gated_bilinear__decode_kernel = build()
```

```python
import functools

import jax
import jax.numpy as jnp
from jax import lax
import jax.experimental.pallas as pl
import jax.experimental.pallas.tpu as pltpu

D = 640
H = 32
DH = 192
SK = 32768
W = 4096
F = 1536
G = 2
NG = H // G
GD = G * DH
EPS = 1e-5

LAG = 24
KW = 2560
KB = 1024
UPI = 2
SPLITS = (1024, 1408, 1536)
NKB = W // KB


def _ln(x):
    m = jnp.mean(x, axis=-1, keepdims=True)
    xc = x - m
    v = jnp.mean(xc * xc, axis=-1, keepdims=True)
    return xc * lax.rsqrt(v + EPS)


def _mm(a, b):
    return jnp.dot(a, b, preferred_element_type=jnp.float32)


def _ds(i, n):
    return pl.ds(pl.multiple_of(i * n, n), n)


def _sweep(i, n, m):
    return lax.rem(i, m) * (n // m) + lax.div(i, m)


def _kernel(x_hbm, c_hbm, kT_hbm, vT_hbm, wq_hbm, wo_hbm, wg_hbm, wu_hbm, wd_hbm, wmod_hbm,
            out_ref,
            x_buf, c_buf, wmod_buf, wq_buf, wo_buf, wg_buf, wu_buf, wd_buf, k_buf, v_buf, mod_buf,
            q_buf, s_buf, hd_buf, ff_buf, t_buf, sem):

    def cols2(src, dst, r, w0, s):
        rows, n = _ds(r, 8), src.shape[1]
        return (pltpu.make_async_copy(src.at[rows, pl.ds(0, w0)], dst.at[rows, pl.ds(0, w0)], s),
                pltpu.make_async_copy(src.at[rows, pl.ds(w0, n - w0)], dst.at[rows, pl.ds(w0, n - w0)], s))

    def rows2(src, dst, r, nr, s):
        a, b = _ds(2 * r, nr), _ds(2 * r + 1, nr)
        return (pltpu.make_async_copy(src.at[a, :], dst.at[a, :], s),
                pltpu.make_async_copy(src.at[b, :], dst.at[b, :], s))

    def u_mod(u):
        return [cols2(wmod_hbm, wmod_buf, _sweep(2 * u + j, 80, 10), 3 * D, sem.at[0]) for j in range(2)]

    def u_wq(u):
        return [cols2(wq_hbm, wq_buf, _sweep(u, 80, 10), H * DH // 2, sem.at[1])]

    def u_wo(u):
        return [rows2(wo_hbm, wo_buf, _sweep(2 * u + j, 128, 16), 24, sem.at[0]) for j in range(2)]

    def u_kv(g, u):
        slot, s = g & 1, sem.at[(g + 1) & 1]
        src_rows, dst_rows = _ds(g * (GD // 8) + u, 8), _ds(u, 8)
        return [(pltpu.make_async_copy(src.at[src_rows, pl.ds(SK - W, KW)],
                                       dst.at[slot, dst_rows, pl.ds(0, KW)], s),
                 pltpu.make_async_copy(src.at[src_rows, pl.ds(SK - W + KW, W - KW)],
                                       dst.at[slot, dst_rows, pl.ds(KW, W - KW)], s))
                for src, dst in ((kT_hbm, k_buf), (vT_hbm, v_buf))]

    def u_ffn(u):
        r = _sweep(u, 40, 4)
        return [rows2(wg_hbm, wg_buf, r, 8, sem.at[1]), rows2(wu_hbm, wu_buf, r, 8, sem.at[1])]

    def start(steps):
        for hi, lo in steps:
            hi.start(priority=0)
            lo.start(priority=1)

    def wait(steps):
        for hi, lo in steps:
            hi.wait()
            lo.wait()

    def pump(old, new, u):
        old, new = old(0), new(u)
        n = max(len(old), len(new))
        for i in range(n):
            wait(old[i * len(old) // n:(i + 1) * len(old) // n])
            start(new[i * len(new) // n:(i + 1) * len(new) // n])

    def pump_loop(lo, hi, old, new):
        if hi > lo:
            @pl.loop(lo, hi)
            def _(u):
                pump(old, new, u)

    small = [pltpu.make_async_copy(x_hbm, x_buf, sem.at[0]), pltpu.make_async_copy(c_hbm, c_buf, sem.at[0])]
    for cp in small:
        cp.start()

    @pl.loop(0, LAG)
    def _(u):
        start(u_mod(u))
    pump_loop(LAG, 40, u_mod, u_mod)

    pump_loop(0, LAG, u_mod, u_wq)
    for cp in small:
        cp.wait()
    x = x_buf[...].astype(jnp.float32)
    c = c_buf[...].astype(jnp.float32)
    sc = jnp.broadcast_to((c * jax.nn.sigmoid(c)).astype(jnp.bfloat16), (8, D))

    @pl.loop(0, 6)
    def _(j):
        pump(u_wq, u_wq, LAG + 2 * j)
        pump(u_wq, u_wq, LAG + 2 * j + 1)
        mod_buf[j] = _mm(sc, wmod_buf[:, _ds(j, D)])
    pump_loop(LAG + 12, 80, u_wq, u_wq)

    pump_loop(0, LAG, u_wq, u_wo)
    h = jnp.broadcast_to((_ln(x) * (1.0 + mod_buf[1][0:1]) + mod_buf[0][0:1]).astype(jnp.bfloat16), (8, D))
    diag = (lax.broadcasted_iota(jnp.int32, (8, GD), 1) // DH) == lax.broadcasted_iota(jnp.int32, (8, GD), 0)

    @pl.loop(0, NG)
    def _(g):
        pump(u_wo, u_wo, LAG + g)
        q_buf[g] = jnp.where(diag, _mm(h, wq_buf[:, _ds(g, GD)]) * (DH ** -0.5), 0.0)
    pump_loop(LAG + NG, 64, u_wo, u_wo)

    kv0 = functools.partial(u_kv, 0)
    pump_loop(0, LAG, u_wo, kv0)
    pump_loop(LAG, 48, kv0, kv0)

    n_pumps = 2 * UPI * NKB + 2

    def attend(g, acc, pump_i):
        slot = g & 1
        qg = q_buf[g].astype(jnp.bfloat16)

        def qk(i, m):
            for t in range(UPI):
                pump_i(UPI * i + t)
            s = _mm(qg, k_buf[slot, :, _ds(i, KB)])
            s_buf[:, _ds(i, KB)] = s
            for j in range(KB // 128):
                m = jnp.maximum(m, s[:, j * 128:(j + 1) * 128])
            return m
        m = lax.fori_loop(0, NKB, qk, jnp.full((8, 128), -jnp.inf, jnp.float32))
        pump_i(UPI * NKB)
        m = jnp.max(m, axis=-1, keepdims=True)

        def pv(i, carry):
            o, l = carry
            for t in range(UPI):
                pump_i(UPI * NKB + 1 + UPI * i + t)
            p = jnp.exp(s_buf[:, _ds(i, KB)] - m)
            for j in range(KB // 128):
                l = l + p[:, j * 128:(j + 1) * 128]
            o = o + lax.dot_general(p.astype(jnp.bfloat16), v_buf[slot, :, _ds(i, KB)],
                                    (((1,), (1,)), ((), ())), preferred_element_type=jnp.float32)
            return o, l
        o, l = lax.fori_loop(0, NKB, pv, (jnp.zeros((8, GD), jnp.float32), jnp.zeros((8, 128), jnp.float32)))
        pump_i(n_pumps - 1)
        l = jnp.sum(l, axis=-1, keepdims=True)
        o = jnp.where(diag, o / l, 0.0).astype(jnp.bfloat16)
        return acc + _mm(o, wo_buf[_ds(g, GD), :])

    def body(g, carry):
        acc, cnt = carry
        new = functools.partial(u_kv, g)
        pump_loop(0, LAG, functools.partial(u_kv, g - 1), new)
        acc = attend(g - 1, acc, lambda i: pump(new, new, LAG + i))
        pump_loop(LAG + n_pumps, 48, new, new)
        return acc, cnt + 1

    acc, cnt = lax.fori_loop(1, NG, body, (jnp.zeros((8, D), jnp.float32), jnp.int32(0)))
    go = cnt == NG - 1

    def ffn_pump(i):
        if isinstance(i, int):
            if LAG + i < 40:
                pump(u_ffn, u_ffn, LAG + i)
        else:
            pl.when(LAG + i < 40)(lambda: pump(u_ffn, u_ffn, LAG + i))

    pump_loop(0, LAG, functools.partial(u_kv, NG - 1), u_ffn)
    acc = attend(NG - 1, acc, ffn_pump)
    x1 = x + mod_buf[2][0:1] * jnp.sum(acc, axis=0, keepdims=True)
    h2 = jnp.broadcast_to((_ln(x1) * (1.0 + mod_buf[4][0:1]) + mod_buf[3][0:1]).astype(jnp.bfloat16), (8, D))
    gb = mod_buf[5][0:1]
    pump_loop(LAG + n_pumps, 40, u_ffn, u_ffn)

    chunks = list(zip((0,) + SPLITS[:-1], SPLITS))

    def wd_copy(i):
        lo, hi = chunks[i]
        return pltpu.make_async_copy(wd_hbm.at[lo:hi, :], wd_buf.at[lo:hi, :], sem.at[i % 2])

    wd_copy(0).start(priority=1)

    @pl.loop(0, LAG)
    def _(u):
        wait(u_ffn(0))
    wd_copy(1).start(priority=1)

    @pl.when(go)
    def _():
        hd_buf[...] = (_mm(h2, wg_buf[...]) * _mm(h2, wu_buf[...])).astype(jnp.bfloat16)

    last_lo, last_hi = chunks[-1]
    nr = last_hi - last_lo

    @pl.when(go)
    def _():
        hl = jnp.broadcast_to(hd_buf[0:1, last_lo:last_hi].astype(jnp.float32), (nr, nr))
        eye = lax.broadcasted_iota(jnp.int32, (nr, nr), 0) == lax.broadcasted_iota(jnp.int32, (nr, nr), 1)
        t_buf[...] = jnp.broadcast_to(jnp.sum(jnp.where(eye, hl, 0.0), axis=1, keepdims=True), (nr, 128))

    for i, (lo, hi) in enumerate(chunks[:-1]):
        wd_copy(i).wait()
        if i + 2 < len(chunks):
            wd_copy(i + 2).start(priority=1)

        @pl.when(go)
        def _():
            ff = _mm(hd_buf[:, lo:hi], wd_buf[lo:hi, :])
            ff_buf[...] = ff if i == 0 else ff_buf[...] + ff

    base = x1 + gb * ff_buf[0:1, :]
    wd_copy(len(chunks) - 1).wait()
    hc = t_buf[...]
    ff = jnp.concatenate(
        [jnp.sum(wd_buf[last_lo:last_hi, j * 128:(j + 1) * 128].astype(jnp.float32) * hc, axis=0, keepdims=True)
         for j in range(D // 128)], axis=1)
    out_ref[...] = (base + gb * ff).astype(out_ref.dtype)


@jax.jit
def pallas_adaLN_cond__sliding_block_cached__glu_gated_bilinear__decode_kernel(
    A_x: jax.Array,
    A_k_cache: jax.Array,
    A_v_cache: jax.Array,
    A_wq: jax.Array,
    A_wo: jax.Array,
    B_x: jax.Array,
    B_w_gate: jax.Array,
    B_w_up: jax.Array,
    B_w_down: jax.Array,
    c: jax.Array,
    w_mod: jax.Array,
):
    del B_x
    kT = jnp.swapaxes(A_k_cache, 2, 3).reshape(H * DH, SK)
    vT = jnp.swapaxes(A_v_cache, 2, 3).reshape(H * DH, SK)
    bf16, f32 = jnp.bfloat16, jnp.float32
    out = pl.pallas_call(
        _kernel,
        in_specs=[pl.BlockSpec(memory_space=pl.ANY)] * 10,
        out_specs=pl.BlockSpec(memory_space=pltpu.VMEM),
        out_shape=jax.ShapeDtypeStruct((1, D), A_x.dtype),
        scratch_shapes=[
            pltpu.VMEM((1, D), bf16), pltpu.VMEM((1, D), bf16),
            pltpu.VMEM((D, 6 * D), bf16), pltpu.VMEM((D, H * DH), bf16), pltpu.VMEM((H * DH, D), bf16),
            pltpu.VMEM((D, F), bf16), pltpu.VMEM((D, F), bf16), pltpu.VMEM((F, D), bf16),
            pltpu.VMEM((2, GD, W), bf16), pltpu.VMEM((2, GD, W), bf16),
            pltpu.VMEM((6, 8, D), f32),
            pltpu.VMEM((NG, 8, GD), f32),
            pltpu.VMEM((8, W), f32),
            pltpu.VMEM((8, F), bf16), pltpu.VMEM((8, D), f32),
            pltpu.VMEM((SPLITS[-1] - SPLITS[-2], 128), f32),
            pltpu.SemaphoreType.DMA((2,)),
        ],
        compiler_params=pltpu.CompilerParams(vmem_limit_bytes=64 * 1024 * 1024),
    )(A_x.reshape(1, D), c, kT, vT, A_wq, A_wo, B_w_gate, B_w_up, B_w_down, w_mod)
    return out.reshape(1, 1, D)
```
